```python
import os as _os
_os.environ.setdefault("JAX_PLATFORMS", "cpu")
import jax
import jax.numpy as jnp

def _softmax(x, axis=-1):
    return jax.nn.softmax(x, axis=axis)
def _gelu(x):
    return jax.nn.gelu(x, approximate=True)
def _silu(x):
    return jax.nn.silu(x)
def _sigmoid(x):
    return jax.nn.sigmoid(x)
def _layernorm(x, axis=-1, eps=1e-5):
    m = jnp.mean(x, axis=axis, keepdims=True)
    v = jnp.var(x, axis=axis, keepdims=True)
    return (x - m) / jnp.sqrt(v + eps)
def _scatter_add(tgt, idx, src, axis=0):
    return tgt.at[idx].add(src)
def _segment_sum(src, seg, n):
    return jax.ops.segment_sum(src, seg, n)
class _Rng:
    def __init__(self, key):
        self._k = key
    def _next(self):
        self._k, sub = jax.random.split(self._k)
        return sub
    def normal(self, shape):
        return jax.random.normal(self._next(), shape, dtype=jnp.bfloat16)
    def randint(self, lo, hi, shape):
        return jax.random.randint(self._next(), shape, lo, hi, dtype=jnp.int32)
    def uniform(self, shape, lo=0.0, hi=1.0):
        return jax.random.uniform(self._next(), shape, jnp.bfloat16, lo, hi)
    def permutation(self, n):
        return jax.random.permutation(self._next(), n)


kernel_name = 'concat_heads__gqa_block_cached__mha_block_cached__near_ridge'

def setup_inputs():
    _rng = _Rng(jax.random.key(int.from_bytes(__import__("os").urandom(4), "little")))
    _w = (lambda a: (lambda t: t.astype(jnp.bfloat16) if jnp.issubdtype(t.dtype, jnp.floating) else t)(jnp.asarray(a)))
    def _A_setup():
        B, Sq, D = 8, 224, 512
        Hq, Hkv, Sk, Dh = 32, 32, 512, 128
        assert Hq % Hkv == 0, (Hq, Hkv)
        return {
            "x": _w((lambda *s: _rng.normal(s) * 0.8)(B, Sq, D)),
            "k_cache": _w((lambda *s: _rng.normal(s) * 0.8)(B, Hkv, Sk, Dh)),
            "v_cache": _w((lambda *s: _rng.normal(s) * 0.05)(B, Hkv, Sk, Dh)),
            "wq": _w((lambda *s: _rng.normal(s) * 0.8)(D, Hq * Dh) * (D ** -0.5)),
            "wo": _w((lambda *s: _rng.normal(s) * 0.05)(Hq * Dh, D) * ((Hq * Dh) ** -0.5)),
        }
    _A_in = _A_setup()

    def _B_setup():
        B, Sq, D = 8, 224, 512
        H, Sk, Dh = 32, 512, 128
        return {
            "x": _w((lambda *s: _rng.normal(s) * 0.8)(B, Sq, D)),
            "k_cache": _w((lambda *s: _rng.normal(s) * 0.8)(B, H, Sk, Dh)),
            "v_cache": _w((lambda *s: _rng.normal(s) * 0.05)(B, H, Sk, Dh)),
            "wq": _w((lambda *s: _rng.normal(s) * 0.8)(D, H * Dh) * (D ** -0.5)),
            "wo": _w((lambda *s: _rng.normal(s) * 0.05)(H * Dh, D) * ((H * Dh) ** -0.5)),
        }
    _B_in = _B_setup()

    return {
        "A_x": _A_in["x"],
        "A_k_cache": _A_in["k_cache"],
        "A_v_cache": _A_in["v_cache"],
        "A_wq": _A_in["wq"],
        "A_wo": _A_in["wo"],
        "B_x": _B_in["x"],
        "B_k_cache": _B_in["k_cache"],
        "B_v_cache": _B_in["v_cache"],
        "B_wq": _B_in["wq"],
        "B_wo": _B_in["wo"],
    }

def reference(A_x, A_k_cache, A_v_cache, A_wq, A_wo, B_x, B_k_cache, B_v_cache, B_wq, B_wo):
    def _A_ref(x, k_cache, v_cache, wq, wo):
        B, Sq, D = x.shape
        Hq, Dh = 32, 128
        Hkv = k_cache.shape[1]
        rep = Hq // Hkv
        q = (lambda x, *d: x.transpose(*d))((x @ wq).reshape(B, Sq, Hq, Dh), 0, 2, 1, 3)
        k = jnp.repeat(k_cache, rep, axis=1)
        v = jnp.repeat(v_cache, rep, axis=1)
        scores = jnp.einsum("bhqd,bhkd->bhqk", q, k) * (Dh ** -0.5)
        p = _softmax(scores, axis=-1)
        o = jnp.einsum("bhqk,bhkd->bhqd", p, v)
        return (lambda x, *d: x.transpose(*d))(o, 0, 2, 1, 3).reshape(B, Sq, Hq * Dh) @ wo

    def _B_ref(x, k_cache, v_cache, wq, wo):
        B, Sq, D = x.shape
        H, Dh = 32, 128
        q = (lambda x, *d: x.transpose(*d))((x @ wq).reshape(B, Sq, H, Dh), 0, 2, 1, 3)
        scores = jnp.einsum("bhqd,bhkd->bhqk", q, k_cache) * (Dh ** -0.5)
        p = _softmax(scores, axis=-1)
        o = jnp.einsum("bhqk,bhkd->bhqd", p, v_cache)
        return (lambda x, *d: x.transpose(*d))(o, 0, 2, 1, 3).reshape(B, Sq, H * Dh) @ wo

    a = _A_ref(A_x, A_k_cache, A_v_cache, A_wq, A_wo)
    b = _B_ref(B_x, B_k_cache, B_v_cache, B_wq, B_wo)
    return jnp.concatenate([a, b], axis=-1)
```

```python
import functools
import jax, jax.numpy as jnp
from jax import lax
import jax.experimental.pallas as pl
import jax.experimental.pallas.tpu as pltpu

B, SQ, D, H, SK, DH = 8, 224, 512, 32, 512, 128
SCALE = DH ** -0.5 * 1.4426950408889634
F32, BF16, U32 = jnp.float32, jnp.bfloat16, jnp.uint32
G = 4
NG = H // G

STRASSEN = {
    1: ({(0,0):1,(1,1):1}, {(0,0):1,(1,1):1}, {(0,0):1,(1,1):1}),
    2: ({(1,0):1,(1,1):1}, {(0,0):1}, {(1,0):1,(1,1):-1}),
    3: ({(0,0):1}, {(0,1):1,(1,1):-1}, {(0,1):1,(1,1):1}),
    4: ({(1,1):1}, {(1,0):1,(0,0):-1}, {(0,0):1,(1,0):1}),
    5: ({(0,0):1,(0,1):1}, {(1,1):1}, {(0,1):1,(0,0):-1}),
    6: ({(1,0):1,(0,0):-1}, {(0,0):1,(0,1):1}, {(1,1):1}),
    7: ({(0,1):1,(1,1):-1}, {(1,0):1,(1,1):1}, {(0,0):1}),
}
QUAD = [(0, 0), (0, 1), (1, 0), (1, 1)]
INTO = {key: {r: t[2][key] for r, t in STRASSEN.items() if key in t[2]} for key in QUAD}

def lincomb(coefs, get):
    acc = None
    for key, c in sorted(coefs.items(), key=lambda kv: -kv[1]):
        v = get(key)
        acc = v if acc is None else acc + v if c == 1 else acc - v
    return acc

def operand(side, load):
    block = functools.cache(load)
    @functools.cache
    def outer(R, i, j):
        return lincomb(STRASSEN[R][side], lambda K: block(2*K[0]+i, 2*K[1]+j))
    return lambda R, r: lincomb(STRASSEN[r][side], lambda k: outer(R, *k))

cols = lambda j, n=1: slice(j*DH, (j+n)*DH)
slot = lambda R, r: 7 * (R - 1) + r - 1
ramp = lambda n, n0, n1, p0, p1: p0 + (p1 - p0) * min(max(n - n0, 0), n1 - n0) / (n1 - n0)

def build(flags='XLA_TPU_RESCHEDULE_DMA_DONES', AHEAD=4, HS=112, PM=0, ORD=0, LAG=1, MIX=0, HEAD=1, TAIL=2, PARTS="pbe",
          OUT=3514726, INN=1457236, INO=1457236, PQ=5, PT=2, P0=13, E0=0, E1=9, E2=13, E3=21, NP=4, WS=1, WS2=2):
    flags = {f: True for f in flags.split("+")} if flags else None
    OUT, INN, INO = ([int(c) for c in str(v)] for v in (OUT, INN, INO))

    def kernel(ax, ak, av, awq, awo, bx, bk, bv, bwq, bwo, out,
               xbuf, kbuf, vbuf, wqbuf, wobuf, xc, mid, obuf, acc, stage, pbuf, zero, sem):
        X, K, V, WQ, WO = (ax, bx), (ak, bk), (av, bv), (awq, bwq), (awo, bwo)
        k32, v32, xc32, p32 = (r.bitcast(U32) for r in (kbuf, vbuf, xc, pbuf))
        zero[0] = 0
        z = zero[0]
        aligned = lambda i, n: i if isinstance(i, int) else pl.multiple_of(i, n)

        def kv_copies(br, s, g, b):
            return [pltpu.make_async_copy(K[br].at[4*s+b, pl.ds(g*G, G)], kbuf.at[br, b], sem.at[4*br+b]),
                    pltpu.make_async_copy(V[br].at[4*s+b, pl.ds(g*G, G)], vbuf.at[br, b], sem.at[8+4*br+b])]
        wq_copy = lambda br, g, J: pltpu.make_async_copy(WQ[br].at[:, pl.ds(aligned((2*g+J) * 2*DH, 2*DH), 2*DH)], wqbuf.at[br, J], sem.at[16+2*br+J])
        wq_copies = lambda br, g: [wq_copy(br, g, 1), wq_copy(br, g, 0)]
        wo_copy = lambda br, g: pltpu.make_async_copy(WO[br].at[pl.ds(aligned(g*G*DH, G*DH), G*DH), :], wobuf.at[br], sem.at[20+br])
        x_copy = lambda br, s, I: pltpu.make_async_copy(X[br].at[pl.ds(4*s+2*I, 2)], xbuf.at[br, pl.ds(2*I, 2)], sem.at[22+2*br+I])
        y_copy = lambda br, s, I, J: pltpu.make_async_copy(stage.at[br, I, J, s], out.at[pl.ds(4*s+2*I, 2), :, pl.ds(br*D + 2*J*DH, 2*DH)], sem.at[26+4*br+2*I+J])

        live = {}; done = set()
        def fold(buf, order, R, r, m):
            live[buf, r] = m
            for n, key in enumerate(QUAD):
                if r == max(INTO[key], key=order.index):
                    mid[z, buf, R-1, n] = lincomb(INTO[key], lambda t: live[buf, t])
        def unfold(buf, i, j):
            return lincomb(INTO[i // 2, j // 2], lambda R: mid[z, buf, R-1, 2*(i % 2) + j % 2])
        def tile_dot(lhs, rhs, split):
            if not split: return jnp.dot(lhs, rhs, preferred_element_type=F32)
            return jnp.concatenate([jnp.dot(part, rhs, preferred_element_type=F32) for part in (lhs[:SQ//2], lhs[SQ//2:])], axis=0)
        def qprod(br, first, R, r, env, split):
            if first and r == INN[0]:
                f = operand(0, lambda i, j: xbuf[br, i, :, cols(j)].astype(F32))
                for t in INN: xc[br, slot(R, t)] = f(R, t).astype(BF16)
            if ("wq", br) not in env: env["wq", br] = operand(1, lambda i, j: wqbuf[br, j // 2, cols(i), cols(j % 2)].astype(F32))
            assert not any(("q", br, t) in done for t in OUT[OUT.index(R):]) or all(("s", br, b, h) in done for b in range(4) for h in range(G) if R in INTO[b // 2, h // 2]), (br, R)
            fold(br, INN, R, r, tile_dot(pltpu.bitcast(xc32[br, slot(R, r)], BF16), env["wq", br](R, r).astype(BF16), split))
            if r == INN[-1]: done.add(("q", br, R))
        def oprod(br, g, s, R, r, env, split):
            for I, J in STRASSEN[R][0]: assert all(("o", br, 2*I+i, 2*J+j) in done for i, j in QUAD), (br, R)
            if ("wo", br) not in env:
                env["wo", br] = operand(1, lambda i, j: wobuf[br, cols(i), cols(j)].astype(F32))
                env["o", br] = operand(0, lambda i, j: obuf[z, br, i, j])
            m = tile_dot(env["o", br](R, r).astype(BF16), env["wo", br](R, r).astype(BF16), split)
            upd = (lambda a: a - m) if PM == 9 else (lambda a: a + m)
            done.add(("y", br, R, r))
            if s is None:
                acc[br, slot(R, r)] = upd(jnp.where(g > 0, acc[br, slot(R, r)], 0.0))
                return
            fold(2, INN, R, r, upd(acc[br, slot(R, r)]))
            for I, J in QUAD:
                if r == INN[-1] and R == max(INTO[I, J], key=OUT.index):
                    for i, j in QUAD:
                        stage[br, I, J, s, i, :, cols(j)] = unfold(2, 2*I+i, 2*J+j).astype(BF16)
                    y_copy(br, s, I, J).start()
        def scores(br, b, h):
            assert all(("q", br, R) in done for R in INTO[b // 2, h // 2]), (br, b, h)
            q = unfold(br, b, h); done.add(("s", br, b, h))
            if "l" in live:
                q = jnp.concatenate([q[:SQ-HS] * jnp.minimum(live.pop("l"), SCALE), q[SQ-HS:] * SCALE], axis=0)
            else:
                q = q * SCALE
            sc = lax.dot_general(q.astype(BF16), pltpu.bitcast(k32[br, b, h], BF16), (((1,), (1,)), ((), ())), preferred_element_type=F32)
            m = jnp.max(sc, axis=-1, keepdims=True)
            if PM == 0: return br, b, h, sc, m
            p = [jnp.exp2(sc[:, cols(j)] - m) for j in range(SK // DH)]
            l = jnp.sum((p[0] + p[1]) + (p[2] + p[3]), axis=-1, keepdims=True)
            r0 = pl.reciprocal(l, approx=True)
            nr = r0 * (l * r0 - 2.0)
            p[0] = jnp.maximum(p[0], nr)
            n = live["n"] = (live.get("n", 0) + 1) % NP
            for j in range(SK // DH): pbuf[z, n, j] = p[j].astype(BF16)
            return br, b, h, n, nr
        def values(br, b, h, sc, m):
            assert ("o", br, b, h) not in done or all(("y", br, R, r) in done for R in OUT for r in OUT if (b // 2, h // 2) in STRASSEN[R][0]), (br, b, h)
            done.add(("o", br, b, h))
            if PM:
                p = jnp.concatenate([pltpu.bitcast(p32[z, sc, j], BF16) for j in range(SK // DH)], axis=1)
                obuf[z, br, b, h] = jnp.dot(p, pltpu.bitcast(v32[br, b, h], BF16), preferred_element_type=F32) * m
                return
            p = [jnp.exp2(sc[:, cols(j)] - m) for j in range(SK // DH)]
            l = jnp.sum((p[0] + p[1]) + (p[2] + p[3]), axis=-1, keepdims=True)
            lo = p[0][:SQ-HS]
            if "l" in live: lo = jnp.minimum(lo, live.pop("l"))
            p[0] = jnp.concatenate([lo, jnp.minimum(p[0][SQ-HS:], l[:HS])], axis=0)
            live["l"] = l[HS:]
            o = jnp.dot(jnp.concatenate(p, axis=1).astype(BF16), pltpu.bitcast(v32[br, b, h], BF16), preferred_element_type=F32)
            obuf[z, br, b, h] = o * pl.reciprocal(l, full_range=False)

        def run(units, queue, target, before, after, ready, half_at=0):
            done.clear(); done.update(ready)
            rounds, k = [], 0
            while k < len(queue):
                n = 2 if len(queue) % 4 and len(rounds) == half_at else 4
                rounds.append(queue[k:k+n]); k += n
            pos = 0
            def upto(n):
                nonlocal pos
                while pos < min(n, len(rounds)) - 1e-6:
                    env = {}
                    for f in rounds[pos]: f(env, len(rounds[pos]) == 2)
                    pos += 1
                    for f in after.get(pos, ()): f()
            pend = []
            for n, u in enumerate(units):
                if ORD != 1 or n == 0: upto(target(n))
                for f in before.get(n, ()): f()
                pend.append(scores(*u))
                if ORD == 1: upto(target(n + 1))
                if ORD == 2: upto((target(n) + target(n + 1)) / 2)
                if len(pend) > LAG: values(*pend.pop(0))
            upto(target(len(units)))
            for u in pend: values(*u)
            upto(len(rounds))
            live.clear()
        Q = lambda br, first=False: [functools.partial(qprod, br, first, R, r) for R in OUT for r in INN]
        O = lambda br, g, s=None: [functools.partial(oprod, br, g, s, R, r) for R in OUT for r in (INO if s is None else INN)]
        heads = lambda br: [(br, b, h) for b in range(4) for h in range(G)]
        held = [("q", 1, R) for R in OUT] + [("o", 0, b, h) for b in range(4) for h in range(G)]

        def kv_sync(waits, starts, chunks, nown):
            hooks = {}
            for c in range(nown):
                ws = list(waits.get(c, ())) + kv_copies(*chunks[c + 1])
                ss = list(starts.get(c, ())) + kv_copies(*chunks[c + AHEAD])
                hooks[4*c + 3] = [x.wait for x in ws] + [x.start for x in ss]
            return hooks
        chunks = lambda *l: [(*t, b) for t in l for b in range(4)]
        def mix(q, o):
            if MIX == 0: return q[:49] + o[:49] + q[49:] + o[49:]
            res = q[:4]; q = q[4:]
            while q or o:
                res += q[:MIX] + o[:MIX]; q = q[MIX:]; o = o[MIX:]
            return res

        def opening(s):
            order = [x_copy(0, s, 0), wq_copy(0, 0, 1) if s == 0 else None, x_copy(0, s, 1), wq_copy(0, 0, 0)]
            for c in range(4):
                order += kv_copies(0, s, 0, c)
                if c == WS: order += [x_copy(1, s, 0), wq_copy(1, 0, 1)]
                if c == WS2: order += [x_copy(1, s, 1), wq_copy(1, 0, 0)]
            return order
        for c in opening(0): c.start()
        x_copy(0, 0, 0).wait(); wq_copy(0, 0, 1).wait()

        def half(s, carry):
            hooks = {}
            for c in range(1, 4):
                kc, vc = kv_copies(0, s, 0, c)
                hooks[4 * c] = [kc.wait]; hooks[4 * c + 1] = [vc.wait]
            later = wq_copies(0, 1) + kv_copies(1, s, 0, 0) + [wo_copy(0, 0)]
            hooks[9] += [c.start for c in later]
            hooks[13] += [c.start for b in (1, 2, 3) for c in kv_copies(1, s, 0, b)]
            kc, vc = kv_copies(0, s, 0, 0)
            hooks[0] = [kc.wait]; hooks[1] = [vc.wait]
            hooks[PQ] = hooks.get(PQ, []) + [x_copy(1, s, 0).wait, wq_copy(1, 0, 1).wait]
            after = {3: [x_copy(0, s, 1).wait, wq_copy(0, 0, 0).wait], 16: [x_copy(1, s, 1).wait, wq_copy(1, 0, 0).wait], 25: [c.wait for c in later]}
            with jax.named_scope("pro"):
              if "p" in PARTS: run(heads(0), Q(0, True) + Q(1, True), lambda n: 12 if n <= PQ else ramp(n, PQ, 16, 12, 25 - PT), hooks, after, [])

            def body(g, carry):
                hooks = kv_sync({2: wq_copies(1, g + 1) + [wo_copy(1, g)], 7: [wq_copy(0, (g + 2) % NG, 1), wq_copy(0, (g + 2) % NG, 0), wo_copy(0, g + 1)]},
                                {4: wq_copies(0, (g + 2) % NG) + [wo_copy(0, g + 1)]},
                                chunks((1, s, g), (0, s, g + 1), (1, s, g + 1)), 8)
                hooks[0] = [c.start for c in wq_copies(1, g + 1) + [wo_copy(1, g)]]
                with jax.named_scope("body"):
                  if "b" in PARTS: run(heads(1) + heads(0), mix(Q(0) + Q(1), O(0, g) + O(1, g)), lambda n: ramp(n, 0, 32, HEAD, 49 - TAIL), hooks, {}, held)
                return carry
            lax.fori_loop(0, NG - 1, body, 0)

            T = NG - 1
            def if_more(copies, op):
                @pl.when(s == 0)
                def _():
                    for c in copies: op(c)
            start, wait = (lambda c: c.start()), (lambda c: c.wait())
            nxt = opening(1)
            hooks = {0: [wo_copy(1, T).start],
                     3: [c.wait for c in kv_copies(1, s, T, 1)] + [functools.partial(if_more, [c for c in nxt[:6] if c is not None], start)],
                     7: [wo_copy(1, T).wait] + [c.wait for c in kv_copies(1, s, T, 2) + kv_copies(1, s, T, 3)] + [functools.partial(if_more, nxt[6:10], start)],
                     15: [functools.partial(if_more, nxt[:1], wait), functools.partial(if_more, nxt[10:], start)]}
            units = heads(1)[:8] + [(1, b, h) for hh in (2, 0) for b in (2, 3) for h in (hh, hh + 1)]
            target = lambda n: ramp(n, 0, E1, E0, 12) if n <= E1 else ramp(n, E1, E2, 12, 15) if n <= E2 else ramp(n, E2, 16, 15, E3 - TAIL)
            with jax.named_scope("epi"):
              if "e" in PARTS: run(units, O(0, T, s) + O(1, T, s), target, hooks, {}, held, half_at=24)
            return carry
        lax.fori_loop(0, 2, half, 0)
        for br in range(2):
            for I, J in QUAD:
                for s in range(2): y_copy(br, s, I, J).wait()

    def fn(A_x, A_k, A_v, A_wq, A_wo, B_x, B_k, B_v, B_wq, B_wo):
        return pl.pallas_call(
            kernel,
            in_specs=[pl.BlockSpec(memory_space=pl.ANY)] * 10,
            out_specs=pl.BlockSpec(memory_space=pl.ANY),
            out_shape=jax.ShapeDtypeStruct((B, SQ, 2 * D), BF16),
            scratch_shapes=[
                pltpu.VMEM((2, 4, SQ, D), BF16),
                pltpu.VMEM((2, 4, G, SK, DH), BF16), pltpu.VMEM((2, 4, G, SK, DH), BF16),
                pltpu.VMEM((2, 2, D, 2 * DH), BF16), pltpu.VMEM((2, G * DH, D), BF16),
                pltpu.VMEM((2, 49, SQ, DH), BF16),
                pltpu.VMEM((2, 3, 7, 4, SQ, DH), F32), pltpu.VMEM((2, 2, 4, G, SQ, DH), F32),
                pltpu.VMEM((2, 49, SQ, DH), F32),
                pltpu.VMEM((2, 2, 2, 2, 2, SQ, 2 * DH), BF16),
                pltpu.VMEM((2, 4, 4, SQ, DH), BF16),
                pltpu.SMEM((1,), jnp.int32),
                pltpu.SemaphoreType.DMA((34,)),
            ],
            compiler_params=pltpu.CompilerParams(vmem_limit_bytes=110 * 2**20, flags=flags, disable_bounds_checks=True),
        )(A_x, A_k, A_v, A_wq, A_wo, B_x, B_k, B_v, B_wq, B_wo)
    return fn


@jax.jit
def pallas_concat_heads__gqa_block_cached__mha_block_cached__near_ridge_kernel(
        A_x, A_k_cache, A_v_cache, A_wq, A_wo, B_x, B_k_cache, B_v_cache, B_wq, B_wo):
    return build()(A_x, A_k_cache, A_v_cache, A_wq, A_wo, B_x, B_k_cache, B_v_cache, B_wq, B_wo)
```

```python
import functools

import jax
import jax.numpy as jnp
from jax import lax
import jax.experimental.pallas as pl
import jax.experimental.pallas.tpu as pltpu

B, SQ, D, H, SK, DH = 8, 224, 512, 32, 512, 128
G = 4
PHASES = H // G
SLOTS = 3
SCALE = DH ** -0.5 * 1.4426950408889634
F32, BF16 = jnp.float32, jnp.bfloat16

STRASSEN = {
    1: ({(0, 0): 1, (1, 1): 1}, {(0, 0): 1, (1, 1): 1}, {(0, 0): 1, (1, 1): 1}),
    2: ({(1, 0): 1, (1, 1): 1}, {(0, 0): 1}, {(1, 0): 1, (1, 1): -1}),
    3: ({(0, 0): 1}, {(0, 1): 1, (1, 1): -1}, {(0, 1): 1, (1, 1): 1}),
    4: ({(1, 1): 1}, {(1, 0): 1, (0, 0): -1}, {(0, 0): 1, (1, 0): 1}),
    5: ({(0, 0): 1, (0, 1): 1}, {(1, 1): 1}, {(0, 1): 1, (0, 0): -1}),
    6: ({(1, 0): 1, (0, 0): -1}, {(0, 0): 1, (0, 1): 1}, {(1, 1): 1}),
    7: ({(0, 1): 1, (1, 1): -1}, {(1, 0): 1, (1, 1): 1}, {(0, 0): 1}),
}
LEFT, RIGHT = 0, 1
QUAD = ((0, 0), (0, 1), (1, 0), (1, 1))
INTO = {c: {r: t[2][c] for r, t in STRASSEN.items() if c in t[2]} for c in QUAD}
SWAP = {r: int(r in (2, 5, 6, 7)) for r in STRASSEN}
WIDE = (1, 6, 7)
Q_LIMIT, Y_LIMIT = 3.0 * 36, 2.0 * 36
COVER = (6, 7)
ROW_LIMIT = 3.0 / SQ
WIDE_PAIRS = sorted(((a, b) for a in WIDE for b in WIDE), key=lambda pair: 1 in pair)

FIRST_ORDER = "ppppppppppppppppppppppppSSVSVSVSVSVSVSVSVSVSVSVSVSVSVSVVp"
LOOP_ORDER = ("pppSSVpppSVSpVSpVpSpVppSVpSVSpVpSpVSpVppSVSpVpppSVpSVpSppVSV"
              "SVpppSVppSVSpVppSVSVSppVpSVSpVpSVpppSVSVpSpVSpVpppSVSpVSVppp"
              "SVSVSpVppSVSppVpSpVSVppSVSpVSpVppSpVpSpVppSVSpVVpp")
LAST_ORDER = "ppSSVSVpSpVppSpVSVSpVpSVpppSVpSVSVpSVpSVpSVppSVpSVppVpppp"
FIRST_Q0, FIRST_Q1 = ("3574126", "6214753"), ("3561472", "2154367")
LOOP_Q = [("5643721", inner) for inner in ("4576213", "4576213", "4752136")]
LOOP_O = [("5364721", inner) for inner in ("6214753", "6214753", "6214753")]
LAST_O6, LAST_O7 = ("5134726", "7453261"), ("5371426", "5317426")


def _signed_sum(signs, get):
    total = None
    for key, sign in sorted(signs.items(), key=lambda item: -item[1]):
        value = get(key)
        total = value if total is None else total + value if sign == 1 else total - value
    return total


def _operands(side, load):
    block = functools.cache(load)

    @functools.cache
    def half(outer, i, j):
        j = j ^ SWAP[outer] if side == RIGHT else j
        return _signed_sum(STRASSEN[outer][side], lambda c: block(2 * c[0] + i, 2 * c[1] + j))

    return lambda outer, inner: _signed_sum(STRASSEN[inner][side], lambda c: half(outer, *c))


def _last(products, order):
    return max(products, key=lambda r: order.index(str(r)))


def _tiles(j, n=1):
    return slice(j * DH, (j + n) * DH)


def _aligned(start, size):
    return pl.ds(start if isinstance(start, int) else pl.multiple_of(start, size), size)


def _energy(value):
    return jnp.sum(value * value, axis=0, keepdims=True)


def _unsafe(mixed, result, limit):
    safe = (mixed > 0.0) & (mixed <= limit * result) & (mixed < jnp.inf)
    return jnp.max(jnp.where(safe, 0.0, 1.0))


def _plain(xs, ks, vs, wqs, wos, out, x, wq, k, v, wo, acc, y, sem):
    @pl.loop(0, 2 * B * H)
    def _(n):
        branch, b, h = n // (B * H), n // H % B, n % H
        head = _aligned(h * DH, DH)
        copies = [(xs, (b,), x), (wqs, (slice(None), head), wq), (ks, (b, h), k),
                  (vs, (b, h), v), (wos, (head,), wo)]
        for side in range(2):
            @pl.when(branch == side)
            def _():
                for c, (sources, index, dst) in enumerate(copies):
                    pltpu.make_async_copy(sources[side].at[index], dst, sem.at[c]).start()
        for c, (_, _, dst) in enumerate(copies):
            pltpu.make_async_copy(dst, dst, sem.at[c]).wait()

        @pl.loop(0, 2)
        def _(half):
            rows = _aligned(half * (SQ // 2), SQ // 2)
            q = (jnp.dot(x[rows], wq[...], preferred_element_type=F32) * SCALE).astype(BF16)
            s = lax.dot_general(q, k[...], (((1,), (1,)), ((), ())), preferred_element_type=F32)
            e = jnp.exp2(s - jnp.max(s, axis=-1, keepdims=True))
            o = jnp.dot(e.astype(BF16), v[...], preferred_element_type=F32)
            o = (o / jnp.sum(e, axis=-1, keepdims=True)).astype(BF16)
            total = jnp.where(h > 0, acc[rows], 0.0) + jnp.dot(
                o, wo[...], preferred_element_type=F32)
            acc[rows] = total
            y[rows] = total.astype(BF16)

        @pl.when(h == H - 1)
        def _():
            copy = pltpu.make_async_copy(y, out.at[b, :, _aligned(branch * D, D)], sem.at[5])
            copy.start()
            copy.wait()


def _kernel(ax, ak, av, awq, awo, bx, bk, bv, bwq, bwo, out,
            x_buf, kv_buf, w_buf, x_ops, halves, o_buf, y_acc, y_buf, p_buf,
            tile_energy, block_energy, row_peak, in_sem, out_sem, *plain_scratch):
    xs, ks, vs, wqs, wos = (ax, bx), (ak, bk), (av, bv), (awq, bwq), (awo, bwo)

    def x_in(rows, i, j):
        dst = x_buf.at[i, j]
        return dst, in_sem.at[i, 7 + j], [
            (xs, (pl.ds(G * rows + 2 * i, 2), slice(None), _tiles(2 * j, 2)), dst)]

    def kv_in(rows, g, slot, b):
        return kv_buf.at[slot, b], in_sem.at[slot, b], [
            (src, (G * rows + b, pl.ds(g * G, G)), kv_buf.at[slot, b, w])
            for w, src in enumerate((ks, vs))]

    def first_kv_in(rows, b, w):
        part = kv_in(rows, 0, 0, b)[2][w]
        return part[2], in_sem.at[0, 9 * w + b], [part]

    def wq_in(g, slot, j):
        dst = w_buf.at[slot, 0, j]
        return dst, in_sem.at[slot, 4 + j], [
            (wqs, (slice(None), _aligned((2 * g + j) * 2 * DH, 2 * DH)), dst)]

    def wo_in(g, slot):
        return w_buf.at[slot, 1], in_sem.at[slot, 6], [
            (wos, (_aligned(g * G * DH, G * DH), _tiles(2 * j, 2)), w_buf.at[slot, 1, j])
            for j in range(2)]

    def start(branch, transfers):
        for _, sem, parts in transfers:
            for side in range(2):
                @pl.when(branch == side)
                def _():
                    for sources, index, dst in parts:
                        pltpu.make_async_copy(sources[side].at[index], dst, sem).start()

    def wait(transfers, when=True):
        @pl.when(when)
        def _():
            for dst, sem, _ in transfers:
                pltpu.make_async_copy(dst, dst, sem).wait()

    popped = {}

    def weights(slot, which):
        return _operands(RIGHT, lambda i, j: w_buf[
            slot, which, j // 2, _tiles(i), _tiles(j % 2)].astype(F32))

    def tile_dot(lhs, rhs, split):
        if not split:
            return jnp.dot(lhs, rhs, preferred_element_type=F32)
        return jnp.concatenate([tile_dot(lhs[:SQ // 2], rhs, False),
                                tile_dot(lhs[SQ // 2:], rhs, False)], axis=0)

    def combine_inner(slot, stage, order, outer, inner, product):
        popped[slot, inner] = product
        if outer in WIDE and inner in WIDE:
            n = WIDE_PAIRS.index((outer, inner))
            tile_energy[stage, n:n + 1] = _energy(product)
        for i, j in QUAD:
            if inner == _last(INTO[i, j], order[1]):
                halves[slot, outer - 1, i, j ^ SWAP[outer]] = _signed_sum(
                    INTO[i, j], lambda r: popped[slot, r])

    def combine_outer(slot, i, j):
        return _signed_sum(INTO[i // 2, j // 2], lambda r: halves[slot, r - 1, i % 2, j % 2])

    def q_product(first, phase, order, outer, inner, shared, split):
        slot, n = phase % SLOTS, 7 * (outer - 1) + inner - 1
        if phase == 0:
            if "x" not in shared:
                shared["x"] = _operands(LEFT, lambda i, j: x_buf[
                    i // 2, j // 2, i % 2, :, _tiles(j % 2)].astype(F32))
            lhs = shared["x"](outer, inner)
            x_ops[n] = lhs.astype(BF16)
            lhs = jnp.concatenate([lhs[:SQ // 2], lhs[SQ // 2:]], axis=0).astype(BF16)
        else:
            lhs = x_ops[n]
        if ("wq", slot) not in shared:
            shared["wq", slot] = weights(slot, 0)
        product = tile_dot(lhs, shared["wq", slot](outer, inner).astype(BF16), split)
        if outer in COVER and inner in COVER:
            n = 2 * COVER.index(outer) + COVER.index(inner)
            peak = jnp.max(jnp.sum(product * product, axis=1, keepdims=True), axis=0, keepdims=True)
            row_peak[first + phase, n:n + 1] = jnp.broadcast_to(peak, (1, DH))
        combine_inner(slot, first + phase, order, outer, inner, product)

    def o_product(phase, keep, quarter, order, outer, inner, shared, split):
        slot, n = phase % SLOTS, 7 * (outer - 1) + inner - 1
        if ("wo", slot) not in shared:
            shared["wo", slot] = weights(slot, 1)
            shared["o", slot] = _operands(LEFT, lambda i, j: o_buf[slot, i, j])
        product = tile_dot(shared["o", slot](outer, inner).astype(BF16),
                           shared["wo", slot](outer, inner).astype(BF16), split)
        total = (y_acc[n] if keep is None else jnp.where(keep, y_acc[n], 0.0)) + product
        if quarter is None:
            y_acc[n] = total
            return
        stage = 4 * PHASES + quarter
        combine_inner(0, stage, order, outer, inner, total)
        for rows, j in QUAD:
            for i in range(2):
                if (outer == _last(INTO[rows, j], order[0])
                        and inner == _last([*INTO[i, 0], *INTO[i, 1]], order[1])):
                    b = 2 * rows + i
                    y = [combine_outer(0, b, 2 * j + c) for c in range(2)]
                    for c in range(2):
                        n = G * b + 2 * j + c
                        block_energy[stage, n:n + 1] = _energy(y[c])
                    y_buf[b, j, quarter] = jnp.concatenate(y, axis=1).astype(BF16)
                    columns = _aligned((quarter // 2) * D + 2 * j * DH, 2 * DH)
                    pltpu.make_async_copy(
                        y_buf.at[b, j, quarter],
                        out.at[G * (quarter % 2) + b, :, columns], out_sem).start()

    def q_products(first, phase, order):
        return [functools.partial(q_product, first, phase, order, int(outer), int(inner))
                for outer in order[0] for inner in order[1]]

    def o_products(phase, order, keep=None, quarter=None):
        return [functools.partial(o_product, phase, keep, quarter, order, int(outer), int(inner))
                for outer in order[0] for inner in order[1]]

    def scores(rows, first, phase, b, h):
        slot = phase % SLOTS
        q = combine_outer(slot, b, h)
        block_energy[first + phase, G * b + h:G * b + h + 1] = _energy(q)
        q = (q * SCALE).astype(BF16)
        s = lax.dot_general(q, kv_buf[slot, b, 0, h], (((1,), (1,)), ((), ())),
                            preferred_element_type=F32)
        top = jnp.max(s, axis=-1, keepdims=True)
        e = [jnp.exp2(s[:, _tiles(j)] - top) for j in range(SK // DH)]
        lanes = (e[0] + e[1]) + (e[2] + e[3])
        e[0] = jnp.minimum(e[0], lanes)
        for j in range(SK // DH):
            p_buf[rows, h % 2, j] = e[j].astype(BF16)
        return phase, b, h, pl.reciprocal(jnp.sum(lanes, axis=-1, keepdims=True), approx=True)

    def values(rows, phase, b, h, inverse):
        slot = phase % SLOTS
        e = jnp.concatenate([p_buf[rows, h % 2, j] for j in range(SK // DH)], axis=1)
        o_buf[slot, b, h] = jnp.dot(
            e, kv_buf[slot, b, 1, h], preferred_element_type=F32) * inverse

    def run(rows, first, order, heads, products, half_round, before_head, product_inputs):
        k, n, rounds, open_heads = 0, 0, 0, []
        for step in order:
            if step == "p":
                size = 2 if rounds == half_round else 4
                for a in range(k, k + size):
                    if a in product_inputs:
                        wait(product_inputs[a])
                shared = {}
                for product in products[k:k + size]:
                    product(shared, size == 2)
                k, rounds = k + size, rounds + 1
            elif step == "S":
                for action in before_head[n]:
                    action()
                open_heads.append(scores(rows, first, *heads[n]))
                n += 1
            else:
                values(rows, *open_heads.pop(0))
        assert n == len(heads) and k == len(products) and not open_heads

    def heads_of(phase):
        return [(phase, b, h) for b in range(G) for h in range(G)]

    def opening(rows):
        return [[x_in(rows, 0, 0), wq_in(0, 0, 1)], [x_in(rows, 0, 1)], [wq_in(1, 1, 1)],
                [x_in(rows, 1, 1), wq_in(0, 0, 0)], [x_in(rows, 1, 0)], [wq_in(1, 1, 0)]]

    def opening_cache(rows):
        return [wq_in(2, 2, 1)] + [first_kv_in(rows, b, w) for b in range(G) for w in range(2)]

    do = functools.partial
    start(0, sum(opening(0), []) + opening_cache(0))
    wait(opening(0)[0])

    @pl.loop(0, 4)
    def _(quarter):
        branch, rows, first = quarter // 2, quarter % 2, quarter * PHASES

        before = [[] for _ in range(16)]
        before[0].append(do(wait, [wq_in(2, 2, 1)]))
        for b in range(G):
            for w in range(2):
                before[G * b + w].append(do(wait, [first_kv_in(rows, b, w)]))
        before[0].append(do(start, branch, [
            wq_in(2, 2, 0), kv_in(rows, 1, 1, 0), kv_in(rows, 1, 1, 1), wo_in(0, 0)]))
        before[12].append(do(start, branch, [kv_in(rows, 1, 1, 2), kv_in(rows, 1, 1, 3)]))
        q0, q1 = q_products(first, 0, FIRST_Q0), q_products(first, 1, FIRST_Q1)
        run(rows, first, FIRST_ORDER, heads_of(0), q0[:14] + q1[:14] + q0[14:] + q1[14:], 0,
            before, dict(zip((7, 14, 28, 49, 63), opening(rows)[1:])))
        wait([wq_in(2, 2, 0)])

        @pl.loop(0, (PHASES - 2) // SLOTS)
        def _(i):
            before = [[] for _ in range(16 * SLOTS)]
            heads, products, inputs = [], [], {}
            start_phase = first + SLOTS * i
            for p in range(1, SLOTS + 1):
                g, n = SLOTS * i + p, 16 * (p - 1)
                more = g + 2 < PHASES if p == SLOTS else True
                next_wq = [wq_in(jnp.minimum(g + 2, PHASES - 1), (p + 2) % SLOTS, j)
                           for j in (1, 0)]
                for b in range(G):
                    before[n + G * b].append(do(wait, [kv_in(rows, g, p % SLOTS, b)]))
                before[n].append(do(start, jnp.where(more, branch, 2), next_wq))
                for b in range(G):
                    before[n + G * b].append(
                        do(start, branch, [kv_in(rows, g + 1, (p + 1) % SLOTS, b)]))
                before[n + G].append(do(start, branch, [wo_in(g, p % SLOTS)]))
                if p == SLOTS:
                    before[n + 15].append(do(wait, next_wq, more))
                    before[n + 15].append(do(wait, [wo_in(g, 0)], g + 2 >= PHASES))
                else:
                    inputs[98 * p] = next_wq
                inputs[98 * p - 49] = [wo_in(g - 1, (p - 1) % SLOTS)]
                heads += heads_of(p)
                products += q_products(start_phase, p + 1, LOOP_Q[p - 1])
                products += o_products(p - 1, LOOP_O[p - 1], keep=i > 0 if p == 1 else None)
            run(rows, start_phase, LOOP_ORDER, heads, products, 0, before, inputs)

        g = PHASES - 1
        next_branch, next_rows = (quarter + 1) // 2, (quarter + 1) % 2
        before = [[] for _ in range(16)]
        for b, n in enumerate((0, 4, 8, 10)):
            before[n].append(do(wait, [kv_in(rows, g, 1, b)]))
        before[0].append(do(start, branch, [wo_in(g, 1)]))
        before[4].append(do(start, next_branch, sum(opening(next_rows), [])))
        before[8].append(do(start, next_branch, opening_cache(next_rows)))
        before[15].append(do(wait, opening(next_rows)[0], next_branch < 2))
        heads = heads_of(g)[:8] + [(g, b, h + c) for h in (2, 0) for b in (2, 3) for c in (0, 1)]
        run(rows, first, LAST_ORDER, heads,
            o_products(g - 1, LAST_O6) + o_products(g, LAST_O7, quarter=quarter), 24, before,
            {49: [wo_in(g, 1)]})

    mixed = jnp.sum(tile_energy[...], axis=1, keepdims=True)
    result = block_energy[...]
    cover = jnp.sum(tile_energy[:4 * PHASES, :4], axis=2, keepdims=True)
    unsafe = (
        _unsafe(mixed[:4 * PHASES], result[:4 * PHASES], Q_LIMIT)
        + _unsafe(row_peak[...], cover, ROW_LIMIT)
        + _unsafe(jnp.sum(mixed[4 * PHASES:], axis=2, keepdims=True),
                  jnp.sum(result[4 * PHASES:], axis=2, keepdims=True), Y_LIMIT))

    written = pltpu.make_async_copy(out, out, out_sem)
    pl.when(unsafe == 0.0)(written.wait)

    @pl.when(unsafe > 0.0)
    def _():
        written.wait()
        _plain(xs, ks, vs, wqs, wos, out, *plain_scratch)


@jax.jit
def pallas_concat_heads__gqa_block_cached__mha_block_cached__near_ridge_kernel(
    A_x: jax.Array,
    A_k_cache: jax.Array,
    A_v_cache: jax.Array,
    A_wq: jax.Array,
    A_wo: jax.Array,
    B_x: jax.Array,
    B_k_cache: jax.Array,
    B_v_cache: jax.Array,
    B_wq: jax.Array,
    B_wo: jax.Array,
):
    return pl.pallas_call(
        _kernel,
        in_specs=[pl.BlockSpec(memory_space=pl.ANY)] * 10,
        out_specs=pl.BlockSpec(memory_space=pl.ANY),
        out_shape=jax.ShapeDtypeStruct((B, SQ, 2 * D), BF16),
        scratch_shapes=[
            pltpu.VMEM((2, 2, 2, SQ, 2 * DH), BF16),
            pltpu.VMEM((SLOTS, G, 2, G, SK, DH), BF16),
            pltpu.VMEM((SLOTS, 2, 2, D, 2 * DH), BF16),
            pltpu.VMEM((49, SQ, DH), BF16),
            pltpu.VMEM((SLOTS, 7, 2, 2, SQ, DH), F32),
            pltpu.VMEM((SLOTS, G, G, SQ, DH), F32),
            pltpu.VMEM((49, SQ, DH), F32),
            pltpu.VMEM((G, 2, 4, SQ, 2 * DH), BF16),
            pltpu.VMEM((2, 2, SK // DH, SQ, DH), BF16),
            pltpu.VMEM((4 * PHASES + 4, 9, DH), F32),
            pltpu.VMEM((4 * PHASES + 4, G * G, DH), F32),
            pltpu.VMEM((4 * PHASES, 4, DH), F32),
            pltpu.SemaphoreType.DMA((SLOTS, 13)),
            pltpu.SemaphoreType.DMA(()),
            pltpu.VMEM((SQ, D), BF16), pltpu.VMEM((D, DH), BF16), pltpu.VMEM((SK, DH), BF16),
            pltpu.VMEM((SK, DH), BF16), pltpu.VMEM((DH, D), BF16), pltpu.VMEM((SQ, D), F32),
            pltpu.VMEM((SQ, D), BF16), pltpu.SemaphoreType.DMA((6,)),
        ],
        compiler_params=pltpu.CompilerParams(
            vmem_limit_bytes=100 * 2**20,
            flags={"XLA_TPU_RESCHEDULE_DMA_DONES": True},
            disable_bounds_checks=True,
            disable_semaphore_checks=True,
        ),
    )(A_x, A_k_cache, A_v_cache, A_wq, A_wo, B_x, B_k_cache, B_v_cache, B_wq, B_wo)
```
